```python
import jax
import jax.numpy as jnp

def _softmax(x, axis=-1):
    return jax.nn.softmax(x, axis=axis)
def _gelu(x):
    return jax.nn.gelu(x, approximate=True)
def _silu(x):
    return jax.nn.silu(x)
def _sigmoid(x):
    return jax.nn.sigmoid(x)
def _layernorm(x, axis=-1, eps=1e-5):
    m = jnp.mean(x, axis=axis, keepdims=True)
    v = jnp.var(x, axis=axis, keepdims=True)
    return (x - m) / jnp.sqrt(v + eps)
def _scatter_add(tgt, idx, src, axis=0):
    return tgt.at[idx].add(src)
def _segment_sum(src, seg, n):
    return jax.ops.segment_sum(src, seg, n)
class _Rng:
    def __init__(self, key):
        self._k = key
    def _next(self):
        self._k, sub = jax.random.split(self._k)
        return sub
    def normal(self, shape):
        return jax.random.normal(self._next(), shape, dtype=jnp.bfloat16)
    def randint(self, lo, hi, shape):
        return jax.random.randint(self._next(), shape, lo, hi, dtype=jnp.int32)
    def uniform(self, shape, lo=0.0, hi=1.0):
        return jax.random.uniform(self._next(), shape, jnp.bfloat16, lo, hi)
    def permutation(self, n):
        return jax.random.permutation(self._next(), n)


kernel_name = 'concat_heads__ssm_conv_h3__compressed_kv_cla__prompt'

def setup_inputs():
    _rng = _Rng(jax.random.key(int.from_bytes(__import__("os").urandom(4), "little")))
    _w = (lambda a: (lambda t: t.astype(jnp.bfloat16) if jnp.issubdtype(t.dtype, jnp.floating) else t)(jnp.asarray(a)))
    def _A_setup():
        B, S, D = 1, 2048, 448
        ks = 4
        return {
            "q": _w((lambda *s: _rng.normal(s) * 0.05)(B, S, D)),
            "k": _w((lambda *s: _rng.normal(s) * 0.05)(B, S, D)),
            "v": _w((lambda *s: _rng.normal(s) * 0.05)(B, S, D)),
            "shift_k": _w((lambda *s: _rng.normal(s) * 0.05)(D, ks) * 0.5),
            "ssm_k": _w((lambda *s: _rng.normal(s) * 0.05)(D, S) * (1.0 / S ** 0.5)),
            "ssm_D": _w((lambda *s: _rng.normal(s) * 0.05)(D)),
        }
    _A_in = _A_setup()

    def _B_setup():
        B, H, Sq, Sk, D, M = 1, 16, 2048, 2048, 256, 448
        Dc = 4 * D
        return {
            "x": _w((lambda *s: _rng.normal(s) * 0.05)(B, Sq, M)),
            "c_kv": _w((lambda *s: _rng.normal(s) * 0.05)(B, Sk, Dc)),
            "w_q": _w((lambda *s: _rng.normal(s) * 0.05)(M, H, D) * (M ** -0.5)),
            "w_uk": _w((lambda *s: _rng.normal(s) * 0.05)(Dc, H, D) * (Dc ** -0.5)),
            "w_uv": _w((lambda *s: _rng.normal(s) * 0.05)(Dc, H, D) * (Dc ** -0.5)),
            "w_o": _w((lambda *s: _rng.normal(s) * 0.05)(H, D, M) * ((H * D) ** -0.5)),
        }
    _B_in = _B_setup()

    return {
        "A_q": _A_in["q"],
        "A_k": _A_in["k"],
        "A_v": _A_in["v"],
        "A_shift_k": _A_in["shift_k"],
        "A_ssm_k": _A_in["ssm_k"],
        "A_ssm_D": _A_in["ssm_D"],
        "B_x": _B_in["x"],
        "B_c_kv": _B_in["c_kv"],
        "B_w_q": _B_in["w_q"],
        "B_w_uk": _B_in["w_uk"],
        "B_w_uv": _B_in["w_uv"],
        "B_w_o": _B_in["w_o"],
    }

def reference(A_q, A_k, A_v, A_shift_k, A_ssm_k, A_ssm_D, B_x, B_c_kv, B_w_q, B_w_uk, B_w_uv, B_w_o):
    def _A_ref(q, k, v, shift_k, ssm_k, ssm_D):
        B, S, D = q.shape
        ks = shift_k.shape[-1]
        k_pad = jnp.pad(k, ((0, 0), (ks - 1, 0), (0, 0)))
        k_shift = jnp.zeros_like(k)
        for t in range(ks):
            k_shift = k_shift + k_pad[:, t:t + S, :] * shift_k[:, ks - 1 - t][None, None, :]
        kv = k_shift * v
        L = 2 * S
        kv_pad = jnp.pad(kv, ((0, 0), (0, S), (0, 0)))
        kf_pad = jnp.pad(ssm_k, ((0, 0), (0, S)))
        kv_f = (lambda x, axes=(-2,-1): jnp.fft.rfft2(x.astype(jnp.float32), axes=axes))(kv_pad[:, None, :, :], axes=(1, 2))
        kf_f = (lambda x, axes=(-2,-1): jnp.fft.rfft2(x.astype(jnp.float32), axes=axes))(kf_pad[:, None, :], axes=(1, 2))
        kf_f = (lambda x, *d: x.transpose(*d))(kf_f, 1, 2, 0)
        y_f = kv_f * kf_f[None, :, :, :]
        y = (lambda x, s, axes=(-2,-1): jnp.fft.irfft2(x, s=s, axes=axes).astype(jnp.bfloat16))(y_f, (1, L), axes=(1, 2))[:, 0, :S, :]
        y = y + kv * ssm_D[None, None, :]
        return q * y

    def _B_ref(x, c_kv, w_q, w_uk, w_uv, w_o):
        B, Sq, M = x.shape[0], x.shape[1], x.shape[2]
        Sk = c_kv.shape[1]
        H, D = w_q.shape[1], w_q.shape[2]
        q = jnp.einsum("bqm,mhd->bhqd", x, w_q)
        k = jnp.einsum("bkc,chd->bhkd", c_kv, w_uk)
        v = jnp.einsum("bkc,chd->bhkd", c_kv, w_uv)
        scores = jnp.einsum("bhqd,bhkd->bhqk", q, k) * (D ** -0.5)
        off = Sk - Sq
        qi = jnp.arange(Sq)[:, None]
        kj = jnp.arange(Sk)[None, :]
        cmask = kj <= (qi + off)
        scores = jnp.where(cmask[None, None], scores, -1e9)
        p = _softmax(scores, axis=-1)
        ctx = jnp.einsum("bhqk,bhkd->bhqd", p, v)
        return jnp.einsum("bhqd,hdm->bqm", ctx, w_o)

    a = _A_ref(A_q, A_k, A_v, A_shift_k, A_ssm_k, A_ssm_D)
    b = _B_ref(B_x, B_c_kv, B_w_q, B_w_uk, B_w_uv, B_w_o)
    return jnp.concatenate([a, b], axis=-1)
```

```python
import numpy as np
import jax
import jax.numpy as jnp
import jax.experimental.pallas as pl
import jax.experimental.pallas.tpu as pltpu

S, DA, H, DH, M, DC = 2048, 448, 16, 256, 448, 1024
N = 2 * S
N1, N2 = 128, 32
BQ = 256
U = 4
BF = jnp.bfloat16
F32 = jnp.float32


def _tables():
    k1 = np.arange(64)[None, :, None] + 0.5
    n = (N2 * np.arange(64)[None, None, :] + np.arange(N2)[:, None, None])
    ang = -2 * np.pi * k1 * n / N
    f1 = np.stack([np.cos(ang), np.sin(ang)], 2).reshape(N2, 128, 64)
    g1 = np.transpose(f1, (0, 2, 1)) * (2.0 / N)
    a = -2 * np.pi * np.outer(np.arange(N2), np.arange(N2)) / N2
    c, s = np.cos(a), np.sin(a)
    f2 = np.zeros((2, 2, N2, 2, 2, N2))
    for p in range(2):
        f2[0, p, :, p, 0], f2[0, p, :, p, 1] = c, -s
        f2[1, p, :, p, 0], f2[1, p, :, p, 1] = s, c
    f2 = f2.reshape(128, 128)
    return f1, g1, f2, f2.T


def _dot(a, b):
    return jnp.dot(a, b, preferred_element_type=F32)


def _ld(ref, r):
    return jnp.concatenate([ref[c, r, :] for c in range(4)], 1)


def _st(ref, r, val):
    for c in range(4):
        ref[c, r, :] = val[:, c * 128:(c + 1) * 128]


def _fwd(src, off, z, f1_ref):
    @pl.loop(0, N2, unroll=U)
    def _(n2):
        xs = _ld(src, pl.ds(off + n2, 64, stride=N2)).astype(BF)
        _st(z, pl.ds(n2, 128, stride=N2), _dot(f1_ref[n2], xs))


def _mixer(q_ref, k_ref, v_ref, sk_ref, kk_ref, d_ref, f1_ref, g1_ref, f2_ref,
           g2_ref, o_ref, tail, u, kt, z, zk):
    u[3] = jnp.zeros(u.shape[1:], F32)
    kt[3] = jnp.zeros(kt.shape[1:], F32)
    for c in range(4):
        w = min(128, DA - c * 128)
        cs = slice(c * 128, c * 128 + w)
        zk[c, 0:8, :] = jnp.zeros((8, 128), F32)
        zk[c, 8:S + 8, 0:w] = k_ref[:, cs].astype(F32)
        sk = sk_ref[:, cs].astype(F32)
        ks = zk[c, 8:S + 8, 0:w] * sk[0:1]
        for j in range(1, 4):
            ks = ks + zk[c, pl.ds(8 - j, S), 0:w] * sk[j:j + 1]
        u[c, :, 0:w] = ks * v_ref[:, cs].astype(F32)
        kt[c, 0:S, 0:w] = kk_ref[cs, :].astype(F32).T
    _fwd(u, 0, z, f1_ref)
    _fwd(kt, 0, zk, f1_ref)
    f2 = f2_ref[...]
    g2 = g2_ref[...]
    @pl.loop(0, 32, unroll=U)
    def _(p):
        r = pl.ds(pl.multiple_of(p * 128, 128), 128)
        a = _dot(f2, _ld(z, r).astype(BF))
        b = _dot(f2, _ld(zk, r).astype(BF))
        ar, ai, br, bi = a[:64], a[64:], b[:64], b[64:]
        pr = jnp.concatenate([ar * br - ai * bi, ar * bi + ai * br], 0)
        _st(z, r, _dot(g2, pr.astype(BF)))
    @pl.loop(0, N2, unroll=U)
    def _(n2):
        zs = _ld(z, pl.ds(n2, 128, stride=N2)).astype(BF)
        _st(kt, pl.ds(n2, 64, stride=N2), _dot(g1_ref[n2], zs))
    tail[...] = jnp.zeros(tail.shape, F32)
    for c in range(4):
        w = min(128, DA - c * 128)
        cs = slice(c * 128, c * 128 + w)
        y = kt[c, :, 0:w] + u[c, :, 0:w] * d_ref[:, cs].astype(F32)
        res = q_ref[:, cs].astype(F32) * y
        if c < 3:
            o_ref[:, cs] = res.astype(BF)
        else:
            tail[:, 0:w] = res


def _head(odd, x_ref, c_ref, wq, wk, wv, wo_ref, acc, qs, ks, vs, cs):
    sh = ((1 - odd) * 16).astype(jnp.uint32)

    def unpack(w):
        bits = (w[...] << sh) & jnp.uint32(0xFFFF0000)
        return pltpu.bitcast(bits, F32).astype(BF)

    qs[...] = (_dot(x_ref[...], unpack(wq)) * (DH ** -0.5)).astype(BF)
    ks[...] = _dot(c_ref[...], unpack(wk)).astype(BF)
    vs[...] = _dot(c_ref[...], unpack(wv)).astype(BF)
    tri = (jax.lax.broadcasted_iota(jnp.int32, (BQ, BQ), 1)
           <= jax.lax.broadcasted_iota(jnp.int32, (BQ, BQ), 0))
    nt = (((1,), (1,)), ((), ()))
    for i in range(S // BQ):
        lo = i * BQ
        q = qs[lo:lo + BQ, :]
        sd = jax.lax.dot_general(q, ks[lo:lo + BQ, :], nt, preferred_element_type=F32)
        sd = jnp.where(tri, sd, -1e9)
        m = jnp.max(sd, axis=1, keepdims=True)
        if i:
            so = jax.lax.dot_general(q, ks[0:lo, :], nt, preferred_element_type=F32)
            m = jnp.maximum(m, jnp.max(so, axis=1, keepdims=True))
            po = jnp.exp(so - m)
        pd = jnp.exp(sd - m)
        l = jnp.sum(pd, axis=1, keepdims=True)
        ctx = _dot(pd.astype(BF), vs[lo:lo + BQ, :])
        if i:
            l = l + jnp.sum(po, axis=1, keepdims=True)
            ctx = ctx + _dot(po.astype(BF), vs[0:lo, :])
        cs[lo:lo + BQ, :] = (ctx / l).astype(BF)
    acc[...] += _dot(cs[...], wo_ref[...])


def _kernel(q_ref, k_ref, v_ref, sk_ref, kk_ref, d_ref, f1_ref, g1_ref, f2_ref,
            g2_ref, x_hbm, c_hbm, wq_hbm, wk_hbm, wv_hbm, wo_ref, o_ref,
            tail, u, kt, z, zk, x_v, c_v, wq_v, wk_v, wv_v, wo_s, acc,
            qs, ks, vs, cs, sem, wsem):
    g = pl.program_id(0)

    def wcopies(hp, slot):
        return [pltpu.make_async_copy(src.bitcast(jnp.uint32).at[:, hp, :],
                                      dst.at[slot], wsem.at[j, slot])
                for j, (src, dst) in enumerate(
                    ((wq_hbm, wq_v), (wk_hbm, wk_v), (wv_hbm, wv_v)))]

    xc = [pltpu.make_async_copy(x_hbm, x_v, sem.at[0]),
          pltpu.make_async_copy(c_hbm, c_v, sem.at[1])]

    @pl.when(g == 0)
    def _():
        for cp in xc + wcopies(0, 0):
            cp.start()
        _mixer(q_ref, k_ref, v_ref, sk_ref, kk_ref, d_ref, f1_ref, g1_ref,
               f2_ref, g2_ref, o_ref, tail, u, kt, z, zk)
        acc[...] = jnp.zeros(acc.shape, F32)
        wo_s[...] = jnp.zeros(wo_s.shape, BF)
        for cp in xc:
            cp.wait()

    @pl.when(g > 0)
    def _():
        h = g - 1
        hp = h // 2
        odd = h % 2
        slot = hp % 2

        @pl.when(odd == 0)
        def _():
            for cp in wcopies(hp, slot):
                cp.wait()

            @pl.when(hp < H // 2 - 1)
            def _():
                for cp in wcopies(hp + 1, 1 - slot):
                    cp.start()

        wo_s[:, 64:512] = wo_ref[0]
        _head(odd, x_v, c_v, wq_v.at[slot], wk_v.at[slot], wv_v.at[slot],
              wo_s, acc, qs, ks, vs, cs)

    @pl.when(g == H)
    def _():
        o_ref[:, 384:512] = (acc[:, 0:128] + tail[...]).astype(BF)
        o_ref[:, 512:896] = acc[:, 128:512].astype(BF)


@jax.jit
def pallas_concat_heads__ssm_conv_h3__compressed_kv_cla__prompt_kernel(
    A_q, A_k, A_v, A_shift_k, A_ssm_k, A_ssm_D,
    B_x, B_c_kv, B_w_q, B_w_uk, B_w_uv, B_w_o,
):
    tabs = [jnp.asarray(t.astype(np.float32).astype(BF)) for t in _tables()]
    vm = pl.BlockSpec(memory_space=pltpu.VMEM)
    hbm = pl.BlockSpec(memory_space=pl.ANY)
    V = pltpu.VMEM
    out = pl.pallas_call(
        _kernel,
        grid=(H + 1,),
        in_specs=[vm] * 10 + [hbm] * 5 + [
            pl.BlockSpec((1, DH, M), lambda g: (jnp.maximum(g - 1, 0), 0, 0))],
        out_specs=pl.BlockSpec((S, 2 * DA), lambda g: (0, 0)),
        out_shape=jax.ShapeDtypeStruct((S, 2 * DA), BF),
        scratch_shapes=[
            V((S, 128), F32), V((4, S, 128), F32), V((4, S, 128), F32),
            V((4, N, 128), F32), V((4, N, 128), F32),
            V((S, M), BF), V((S, DC), BF),
            V((2, M, DH), jnp.uint32), V((2, DC, DH), jnp.uint32),
            V((2, DC, DH), jnp.uint32), V((DH, 512), BF), V((S, 512), F32),
            V((S, DH), BF), V((S, DH), BF), V((S, DH), BF), V((S, DH), BF),
            pltpu.SemaphoreType.DMA((2,)), pltpu.SemaphoreType.DMA((3, 2)),
        ],
        compiler_params=pltpu.CompilerParams(
            dimension_semantics=("arbitrary",),
            vmem_limit_bytes=110 * 1024 * 1024),
    )(A_q[0], A_k[0], A_v[0], A_shift_k.T, A_ssm_k, A_ssm_D[None, :], *tabs,
      B_x[0], B_c_kv[0], B_w_q, B_w_uk, B_w_uv, B_w_o)
    return out[None]
```

```python
import numpy as np
import jax
import jax.numpy as jnp
import jax.experimental.pallas as pl
import jax.experimental.pallas.tpu as pltpu

S, DA, H, DH, M, DC = 2048, 448, 16, 256, 448, 1024
N = 2 * S
N1, N2 = 128, 32
BQ = 256
U = 4
BF = jnp.bfloat16
F32 = jnp.float32


def _tables():
    k1 = np.arange(64)[None, :, None] + 0.5
    n = (N2 * np.arange(64)[None, None, :] + np.arange(N2)[:, None, None])
    ang = -2 * np.pi * k1 * n / N
    f1 = np.stack([np.cos(ang), np.sin(ang)], 2).reshape(N2, 128, 64)
    g1 = np.transpose(f1, (0, 2, 1)) * (2.0 / N)
    a = -2 * np.pi * np.outer(np.arange(N2), np.arange(N2)) / N2
    c, s = np.cos(a), np.sin(a)
    f2 = np.zeros((2, 2, N2, 2, 2, N2))
    for p in range(2):
        f2[0, p, :, p, 0], f2[0, p, :, p, 1] = c, -s
        f2[1, p, :, p, 0], f2[1, p, :, p, 1] = s, c
    f2 = f2.reshape(128, 128)
    return f1, g1, f2, f2.T


def _dot(a, b):
    return jnp.dot(a, b, preferred_element_type=F32)


def _ld(ref, r):
    return jnp.concatenate([ref[c, r, :] for c in range(4)], 1)


def _st(ref, r, val):
    for c in range(4):
        ref[c, r, :] = val[:, c * 128:(c + 1) * 128]


def _fwd(src, off, z, f1_ref):
    @pl.loop(0, N2, unroll=U)
    def _(n2):
        xs = _ld(src, pl.ds(off + n2, 64, stride=N2)).astype(BF)
        _st(z, pl.ds(n2, 128, stride=N2), _dot(f1_ref[n2], xs))


def _mixer(q_ref, k_ref, v_ref, sk_ref, kk_ref, d_ref, f1_ref, g1_ref, f2_ref,
           g2_ref, o_ref, tail, u, kt, z, zk):
    u[3] = jnp.zeros(u.shape[1:], F32)
    kt[3] = jnp.zeros(kt.shape[1:], F32)
    for c in range(4):
        w = min(128, DA - c * 128)
        cs = slice(c * 128, c * 128 + w)
        zk[c, 0:8, :] = jnp.zeros((8, 128), F32)
        zk[c, 8:S + 8, 0:w] = k_ref[cs, :].astype(F32).T
        sk = sk_ref[:, cs].astype(F32)
        ks = zk[c, 8:S + 8, 0:w] * sk[0:1]
        for j in range(1, 4):
            ks = ks + zk[c, pl.ds(8 - j, S), 0:w] * sk[j:j + 1]
        u[c, :, 0:w] = ks * v_ref[cs, :].astype(F32).T
        kt[c, 0:S, 0:w] = kk_ref[cs, :].astype(F32).T
    _fwd(u, 0, z, f1_ref)
    _fwd(kt, 0, zk, f1_ref)
    f2 = f2_ref[...]
    g2 = g2_ref[...]
    @pl.loop(0, 32, unroll=U)
    def _(p):
        r = pl.ds(pl.multiple_of(p * 128, 128), 128)
        a = _dot(f2, _ld(z, r).astype(BF))
        b = _dot(f2, _ld(zk, r).astype(BF))
        ar, ai, br, bi = a[:64], a[64:], b[:64], b[64:]
        pr = jnp.concatenate([ar * br - ai * bi, ar * bi + ai * br], 0)
        _st(z, r, _dot(g2, pr.astype(BF)))
    @pl.loop(0, N2, unroll=U)
    def _(n2):
        zs = _ld(z, pl.ds(n2, 128, stride=N2)).astype(BF)
        _st(kt, pl.ds(n2, 64, stride=N2), _dot(g1_ref[n2], zs))
    tail[...] = jnp.zeros(tail.shape, F32)
    for c in range(4):
        w = min(128, DA - c * 128)
        cs = slice(c * 128, c * 128 + w)
        y = kt[c, :, 0:w] + u[c, :, 0:w] * d_ref[:, cs].astype(F32)
        res = q_ref[cs, :].astype(F32).T * y
        if c < 3:
            o_ref[:, cs] = res.astype(BF)
        else:
            tail[:, 0:w] = res


def _head(odd, x_ref, c_ref, wq, wk, wv, wo_ref, acc, qs, ks, vs, cs):
    sh = ((1 - odd) * 16).astype(jnp.uint32)

    def unpack(w):
        bits = (w[...] << sh) & jnp.uint32(0xFFFF0000)
        return pltpu.bitcast(bits, F32).astype(BF)

    qs[...] = (_dot(x_ref[...], unpack(wq)) * (DH ** -0.5)).astype(BF)
    ks[...] = _dot(c_ref[...], unpack(wk)).astype(BF)
    vs[...] = _dot(c_ref[...], unpack(wv)).astype(BF)
    tri = (jax.lax.broadcasted_iota(jnp.int32, (BQ, BQ), 1)
           <= jax.lax.broadcasted_iota(jnp.int32, (BQ, BQ), 0))
    nt = (((1,), (1,)), ((), ()))
    for i in range(S // BQ):
        lo = i * BQ
        q = qs[lo:lo + BQ, :]
        sd = jax.lax.dot_general(q, ks[lo:lo + BQ, :], nt, preferred_element_type=F32)
        sd = jnp.where(tri, sd, -1e9)
        m = jnp.max(sd, axis=1, keepdims=True)
        if i:
            so = jax.lax.dot_general(q, ks[0:lo, :], nt, preferred_element_type=F32)
            m = jnp.maximum(m, jnp.max(so, axis=1, keepdims=True))
            po = jnp.exp(so - m)
        pd = jnp.exp(sd - m)
        l = jnp.sum(pd, axis=1, keepdims=True)
        ctx = _dot(pd.astype(BF), vs[lo:lo + BQ, :])
        if i:
            l = l + jnp.sum(po, axis=1, keepdims=True)
            ctx = ctx + _dot(po.astype(BF), vs[0:lo, :])
        cs[lo:lo + BQ, :] = (ctx / l).astype(BF)
    acc[...] += jax.lax.dot_general(cs[...], wo_ref[...], nt, preferred_element_type=F32)


def _kernel(q_ref, k_ref, v_ref, sk_ref, kk_ref, d_ref, f1_ref, g1_ref, f2_ref,
            g2_ref, x_hbm, c_hbm, wq_hbm, wk_hbm, wv_hbm, wo_ref, o_ref,
            tail, u, kt, z, zk, xt, x_v, c_v, wq_v, wk_v, wv_v, wo_s, acc,
            qs, ks, vs, cs, sem, wsem):
    g = pl.program_id(0)

    def wcopies(hp, slot):
        return [pltpu.make_async_copy(src.bitcast(jnp.uint32).at[:, hp, :],
                                      dst.at[slot], wsem.at[j, slot])
                for j, (src, dst) in enumerate(
                    ((wq_hbm, wq_v), (wk_hbm, wk_v), (wv_hbm, wv_v)))]

    xc = [pltpu.make_async_copy(x_hbm, xt, sem.at[0]),
          pltpu.make_async_copy(c_hbm, c_v, sem.at[1])]

    @pl.when(g == 0)
    def _():
        for cp in xc + wcopies(0, 0):
            cp.start()
        _mixer(q_ref, k_ref, v_ref, sk_ref, kk_ref, d_ref, f1_ref, g1_ref,
               f2_ref, g2_ref, o_ref, tail, u, kt, z, zk)
        acc[...] = jnp.zeros(acc.shape, F32)
        wo_s[...] = jnp.zeros(wo_s.shape, BF)
        for cp in xc:
            cp.wait()
        for c in range(0, M, 128):
            e = min(M, c + 128)
            x_v[:, c:e] = xt[c:e, :].astype(F32).T.astype(BF)

    @pl.when(g > 0)
    def _():
        h = g - 1
        hp = h // 2
        odd = h % 2
        slot = hp % 2

        @pl.when(odd == 0)
        def _():
            for cp in wcopies(hp, slot):
                cp.wait()

            @pl.when(hp < H // 2 - 1)
            def _():
                for cp in wcopies(hp + 1, 1 - slot):
                    cp.start()

        wo_s[64:512, :] = wo_ref[0]
        _head(odd, x_v, c_v, wq_v.at[slot], wk_v.at[slot], wv_v.at[slot],
              wo_s, acc, qs, ks, vs, cs)

    @pl.when(g == H)
    def _():
        o_ref[:, 384:512] = (acc[:, 0:128] + tail[...]).astype(BF)
        o_ref[:, 512:896] = acc[:, 128:512].astype(BF)


@jax.jit
def pallas_concat_heads__ssm_conv_h3__compressed_kv_cla__prompt_kernel(
    A_q, A_k, A_v, A_shift_k, A_ssm_k, A_ssm_D,
    B_x, B_c_kv, B_w_q, B_w_uk, B_w_uv, B_w_o,
):
    tabs = [jnp.asarray(t.astype(np.float32).astype(BF)) for t in _tables()]
    vm = pl.BlockSpec(memory_space=pltpu.VMEM)
    hbm = pl.BlockSpec(memory_space=pl.ANY)
    V = pltpu.VMEM
    out = pl.pallas_call(
        _kernel,
        grid=(H + 1,),
        in_specs=[vm] * 10 + [hbm] * 5 + [
            pl.BlockSpec((1, M, DH), lambda g: (jnp.maximum(g - 1, 0), 0, 0))],
        out_specs=pl.BlockSpec((S, 2 * DA), lambda g: (0, 0)),
        out_shape=jax.ShapeDtypeStruct((S, 2 * DA), BF),
        scratch_shapes=[
            V((S, 128), F32), V((4, S, 128), F32), V((4, S, 128), F32),
            V((4, N, 128), F32), V((4, N, 128), F32),
            V((M, S), BF), V((S, M), BF), V((S, DC), BF),
            V((2, M, DH), jnp.uint32), V((2, DC, DH), jnp.uint32),
            V((2, DC, DH), jnp.uint32), V((512, DH), BF), V((S, 512), F32),
            V((S, DH), BF), V((S, DH), BF), V((S, DH), BF), V((S, DH), BF),
            pltpu.SemaphoreType.DMA((2,)), pltpu.SemaphoreType.DMA((3, 2)),
        ],
        compiler_params=pltpu.CompilerParams(
            dimension_semantics=("arbitrary",),
            vmem_limit_bytes=110 * 1024 * 1024),
    )(A_q[0].T, A_k[0].T, A_v[0].T, A_shift_k.T, A_ssm_k, A_ssm_D[None, :], *tabs,
      B_x[0].T, B_c_kv[0], B_w_q, B_w_uk, B_w_uv, B_w_o.transpose(0, 2, 1))
    return out[None]
```

```python
import numpy as np
import jax
import jax.numpy as jnp
import jax.experimental.pallas as pl
import jax.experimental.pallas.tpu as pltpu

S, DA, H, DH, M, DC = 2048, 448, 16, 256, 448, 1024
N = 2 * S
N1, N2 = 128, 32
BQ = 256
BF = jnp.bfloat16
F32 = jnp.float32


def _tables():
    k1 = np.arange(64)[None, :, None] + 0.5
    n = (N2 * np.arange(64)[None, None, :] + np.arange(N2)[:, None, None])
    ang = -2 * np.pi * k1 * n / N
    f1 = np.stack([np.cos(ang), np.sin(ang)], 2).reshape(N2, 128, 64)
    g1 = np.transpose(f1, (0, 2, 1)) * (2.0 / N)
    a = -2 * np.pi * np.outer(np.arange(N2), np.arange(N2)) / N2
    c, s = np.cos(a), np.sin(a)
    f2 = np.zeros((2, 2, N2, 2, 2, N2))
    for p in range(2):
        f2[0, p, :, p, 0], f2[0, p, :, p, 1] = c, -s
        f2[1, p, :, p, 0], f2[1, p, :, p, 1] = s, c
    f2 = f2.reshape(128, 128)
    return f1, g1, f2, f2.T


def _dot(a, b):
    return jnp.dot(a, b, preferred_element_type=F32)


def _ld(ref, r):
    return jnp.concatenate([ref[c, r, :] for c in range(4)], 1)


def _st(ref, r, val):
    for c in range(4):
        ref[c, r, :] = val[:, c * 128:(c + 1) * 128]


def _fwd(src, off, z, f1_ref):
    @pl.loop(0, N2, unroll=8)
    def _(n2):
        xs = _ld(src, pl.ds(off + n2, 64, stride=N2)).astype(BF)
        _st(z, pl.ds(n2, 128, stride=N2), _dot(f1_ref[n2], xs))


def _mixer(q_ref, k_ref, v_ref, sk_ref, kk_ref, d_ref, f1_ref, g1_ref, f2_ref,
           g2_ref, o_ref, tail, u, kt, z, zk):
    u[3] = jnp.zeros(u.shape[1:], F32)
    kt[3] = jnp.zeros(kt.shape[1:], F32)
    for c in range(4):
        w = min(128, DA - c * 128)
        cs = slice(c * 128, c * 128 + w)
        zk[c, 0:8, :] = jnp.zeros((8, 128), F32)
        zk[c, 8:S + 8, 0:w] = k_ref[cs, :].astype(F32).T
        sk = sk_ref[:, cs].astype(F32)
        ks = zk[c, 8:S + 8, 0:w] * sk[0:1]
        for j in range(1, 4):
            ks = ks + zk[c, pl.ds(8 - j, S), 0:w] * sk[j:j + 1]
        u[c, :, 0:w] = ks * v_ref[cs, :].astype(F32).T
        kt[c, 0:S, 0:w] = kk_ref[cs, :].astype(F32).T
    _fwd(u, 0, z, f1_ref)
    _fwd(kt, 0, zk, f1_ref)
    f2 = f2_ref[...]
    g2 = g2_ref[...]
    @pl.loop(0, 32, unroll=2)
    def _(p):
        r = pl.ds(pl.multiple_of(p * 128, 128), 128)
        a = _dot(f2, _ld(z, r).astype(BF))
        b = _dot(f2, _ld(zk, r).astype(BF))
        ar, ai, br, bi = a[:64], a[64:], b[:64], b[64:]
        pr = jnp.concatenate([ar * br - ai * bi, ar * bi + ai * br], 0)
        _st(z, r, _dot(g2, pr.astype(BF)))
    @pl.loop(0, N2, unroll=8)
    def _(n2):
        zs = _ld(z, pl.ds(n2, 128, stride=N2)).astype(BF)
        _st(kt, pl.ds(n2, 64, stride=N2), _dot(g1_ref[n2], zs))
    tail[...] = jnp.zeros(tail.shape, F32)
    for c in range(4):
        w = min(128, DA - c * 128)
        cs = slice(c * 128, c * 128 + w)
        y = kt[c, :, 0:w] + u[c, :, 0:w] * d_ref[:, cs].astype(F32)
        res = q_ref[cs, :].astype(F32).T * y
        if c < 3:
            o_ref[:, cs] = res.astype(BF)
        else:
            tail[:, 0:w] = res


def _head(odd, x_ref, c_ref, wq, wk, wv, wo_ref, acc, qs, ks, vs, cs):
    sh = ((1 - odd) * 16).astype(jnp.uint32)

    def unpack(w):
        bits = (w[...] << sh) & jnp.uint32(0xFFFF0000)
        return pltpu.bitcast(bits, F32).astype(BF)

    qs[...] = (_dot(x_ref[...], unpack(wq)) * (DH ** -0.5)).astype(BF)
    ks[...] = _dot(c_ref[...], unpack(wk)).astype(BF)
    vs[...] = _dot(c_ref[...], unpack(wv)).astype(BF)
    tri = (jax.lax.broadcasted_iota(jnp.int32, (BQ, BQ), 1)
           <= jax.lax.broadcasted_iota(jnp.int32, (BQ, BQ), 0))
    nt = (((1,), (1,)), ((), ()))
    for i in range(S // BQ):
        lo = i * BQ
        q = qs[lo:lo + BQ, :]
        s0 = jax.lax.dot_general(q, ks[lo:lo + 128, :], nt, preferred_element_type=F32)
        s1 = jax.lax.dot_general(q[128:], ks[lo + 128:lo + BQ, :], nt, preferred_element_type=F32)
        sd = jnp.concatenate([s0, jnp.concatenate([s0[:128], s1], 0)], 1)
        sd = jnp.where(tri, sd, -1e9)
        m = jnp.max(sd, axis=1, keepdims=True)
        if i:
            so = jax.lax.dot_general(q, ks[0:lo, :], nt, preferred_element_type=F32)
            m = jnp.maximum(m, jnp.max(so, axis=1, keepdims=True))
            po = jnp.exp(so - m)
        pd = jnp.exp(sd - m)
        l = jnp.sum(pd, axis=1, keepdims=True)
        pb = pd.astype(BF)
        ctx = _dot(pb[:, :128], vs[lo:lo + 128, :])
        c1 = _dot(pb[128:, 128:], vs[lo + 128:lo + BQ, :])
        ctx = jnp.concatenate([ctx[:128], ctx[128:] + c1], 0)
        if i:
            l = l + jnp.sum(po, axis=1, keepdims=True)
            ctx = ctx + _dot(po.astype(BF), vs[0:lo, :])
        cs[lo:lo + BQ, :] = (ctx / l).astype(BF)
    acc[...] += jax.lax.dot_general(cs[...], wo_ref[...], nt, preferred_element_type=F32)


def _kernel(q_ref, k_ref, v_ref, sk_ref, kk_ref, d_ref, f1_ref, g1_ref, f2_ref,
            g2_ref, x_hbm, c_hbm, wq_hbm, wk_hbm, wv_hbm, wo_ref, o_ref,
            tail, u, kt, z, zk, xt, x_v, c_v, wq_v, wk_v, wv_v, wo_s, acc,
            qs, ks, vs, cs, sem, wsem):
    g = pl.program_id(0)

    def wcopies(hp, slot):
        return [pltpu.make_async_copy(src.bitcast(jnp.uint32).at[:, hp, :],
                                      dst.at[slot], wsem.at[j, slot])
                for j, (src, dst) in enumerate(
                    ((wq_hbm, wq_v), (wk_hbm, wk_v), (wv_hbm, wv_v)))]

    xc = [pltpu.make_async_copy(x_hbm, xt, sem.at[0]),
          pltpu.make_async_copy(c_hbm, c_v, sem.at[1])]

    @pl.when(g == 0)
    def _():
        for cp in xc + wcopies(0, 0):
            cp.start()
        _mixer(q_ref, k_ref, v_ref, sk_ref, kk_ref, d_ref, f1_ref, g1_ref,
               f2_ref, g2_ref, o_ref, tail, u, kt, z, zk)
        acc[...] = jnp.zeros(acc.shape, F32)
        wo_s[...] = jnp.zeros(wo_s.shape, BF)
        for cp in xc:
            cp.wait()
        for c in range(0, M, 128):
            e = min(M, c + 128)
            x_v[:, c:e] = xt[c:e, :].astype(F32).T.astype(BF)

    @pl.when(g > 0)
    def _():
        h = g - 1
        hp = h // 2
        odd = h % 2
        slot = hp % 2

        @pl.when(odd == 0)
        def _():
            for cp in wcopies(hp, slot):
                cp.wait()

            @pl.when(hp < H // 2 - 1)
            def _():
                for cp in wcopies(hp + 1, 1 - slot):
                    cp.start()

        wo_s[64:512, :] = wo_ref[0]
        _head(odd, x_v, c_v, wq_v.at[slot], wk_v.at[slot], wv_v.at[slot],
              wo_s, acc, qs, ks, vs, cs)

    @pl.when(g == H)
    def _():
        o_ref[:, 384:512] = (acc[:, 0:128] + tail[...]).astype(BF)
        o_ref[:, 512:896] = acc[:, 128:512].astype(BF)


@jax.jit
def pallas_concat_heads__ssm_conv_h3__compressed_kv_cla__prompt_kernel(
    A_q, A_k, A_v, A_shift_k, A_ssm_k, A_ssm_D,
    B_x, B_c_kv, B_w_q, B_w_uk, B_w_uv, B_w_o,
):
    tabs = [jnp.asarray(t.astype(np.float32).astype(BF)) for t in _tables()]
    vm = pl.BlockSpec(memory_space=pltpu.VMEM)
    hbm = pl.BlockSpec(memory_space=pl.ANY)
    V = pltpu.VMEM
    out = pl.pallas_call(
        _kernel,
        grid=(H + 1,),
        in_specs=[vm] * 10 + [hbm] * 5 + [
            pl.BlockSpec((1, M, DH), lambda g: (jnp.maximum(g - 1, 0), 0, 0))],
        out_specs=pl.BlockSpec((S, 2 * DA), lambda g: (0, 0)),
        out_shape=jax.ShapeDtypeStruct((S, 2 * DA), BF),
        scratch_shapes=[
            V((S, 128), F32), V((4, S, 128), F32), V((4, S, 128), F32),
            V((4, N, 128), F32), V((4, N, 128), F32),
            V((M, S), BF), V((S, M), BF), V((S, DC), BF),
            V((2, M, DH), jnp.uint32), V((2, DC, DH), jnp.uint32),
            V((2, DC, DH), jnp.uint32), V((512, DH), BF), V((S, 512), F32),
            V((S, DH), BF), V((S, DH), BF), V((S, DH), BF), V((S, DH), BF),
            pltpu.SemaphoreType.DMA((2,)), pltpu.SemaphoreType.DMA((3, 2)),
        ],
        compiler_params=pltpu.CompilerParams(
            dimension_semantics=("arbitrary",),
            vmem_limit_bytes=110 * 1024 * 1024),
    )(A_q[0].T, A_k[0].T, A_v[0].T, A_shift_k.T, A_ssm_k, A_ssm_D[None, :], *tabs,
      B_x[0].T, B_c_kv[0], B_w_q, B_w_uk, B_w_uv, B_w_o.transpose(0, 2, 1))
    return out[None]
```
